```python
import jax
import jax.numpy as jnp

def _softmax(x, axis=-1):
    return jax.nn.softmax(x, axis=axis)
def _gelu(x):
    return jax.nn.gelu(x, approximate=True)
def _silu(x):
    return jax.nn.silu(x)
def _sigmoid(x):
    return jax.nn.sigmoid(x)
def _layernorm(x, axis=-1, eps=1e-5):
    m = jnp.mean(x, axis=axis, keepdims=True)
    v = jnp.var(x, axis=axis, keepdims=True)
    return (x - m) / jnp.sqrt(v + eps)
def _scatter_add(tgt, idx, src, axis=0):
    return tgt.at[idx].add(src)
def _segment_sum(src, seg, n):
    return jax.ops.segment_sum(src, seg, n)
class _Rng:
    def __init__(self, key):
        self._k = key
    def _next(self):
        self._k, sub = jax.random.split(self._k)
        return sub
    def normal(self, shape):
        return jax.random.normal(self._next(), shape, dtype=jnp.bfloat16)
    def randint(self, lo, hi, shape):
        return jax.random.randint(self._next(), shape, lo, hi, dtype=jnp.int32)
    def uniform(self, shape, lo=0.0, hi=1.0):
        return jax.random.uniform(self._next(), shape, jnp.bfloat16, lo, hi)
    def permutation(self, n):
        return jax.random.permutation(self._next(), n)


kernel_name = 'recurrent_scan__sliding_block_cached__glu_gated_swiglu__decode'

def setup_inputs():
    _rng = _Rng(jax.random.key(int.from_bytes(__import__("os").urandom(4), "little")))
    _w = (lambda a: (lambda t: t.astype(jnp.bfloat16) if jnp.issubdtype(t.dtype, jnp.floating) else t)(jnp.asarray(a)))
    def _A_setup():
        B, Sq, D = 1, 1, 640
        Hq, Hkv, Sk, Dh = 32, 32, 32768, 192
        assert Hq % Hkv == 0, (Hq, Hkv)
        return {
            "x": _w((lambda *s: _rng.normal(s) * 0.05)(B, Sq, D)),
            "k_cache": _w((lambda *s: _rng.normal(s) * 0.05)(B, Hkv, Sk, Dh)),
            "v_cache": _w((lambda *s: _rng.normal(s) * 0.05)(B, Hkv, Sk, Dh)),
            "wq": _w((lambda *s: _rng.normal(s) * 0.05)(D, Hq * Dh) * (D ** -0.5)),
            "wo": _w((lambda *s: _rng.normal(s) * 0.05)(Hq * Dh, D) * ((Hq * Dh) ** -0.5)),
        }
    _A_in = _A_setup()

    def _B_setup():
        B, S, D, F = 1, 1, 640, 1536
        return {
            "x": _w((lambda *s: _rng.normal(s) * 0.05)(B, S, D)),
            "w1": _w((lambda *s: _rng.normal(s) * 0.05)(D, F) * (2.0 / D) ** 0.5),
            "w3": _w((lambda *s: _rng.normal(s) * 0.05)(D, F) * (2.0 / D) ** 0.5),
            "w2": _w((lambda *s: _rng.normal(s) * 0.05)(F, D) * (2.0 / F) ** 0.5),
        }
    _B_in = _B_setup()

    return {
        "A_x": _A_in["x"],
        "A_k_cache": _A_in["k_cache"],
        "A_v_cache": _A_in["v_cache"],
        "A_wq": _A_in["wq"],
        "A_wo": _A_in["wo"],
        "B_x": _B_in["x"],
        "B_w1": _B_in["w1"],
        "B_w3": _B_in["w3"],
        "B_w2": _B_in["w2"],
    }

def reference(A_x, A_k_cache, A_v_cache, A_wq, A_wo, B_x, B_w1, B_w3, B_w2):
    def _A_ref(x, k_cache, v_cache, wq, wo):
        B, Sq, D = x.shape
        Hq, Dh = 32, 192
        Hkv, Sk = k_cache.shape[1], k_cache.shape[2]
        W = min(4096, max(256, Sk // 4))
        rep = Hq // Hkv
        q = (lambda x, *d: x.transpose(*d))((x @ wq).reshape(B, Sq, Hq, Dh), 0, 2, 1, 3)
        k = jnp.repeat(k_cache[:, :, Sk - W:, :], rep, axis=1)
        v = jnp.repeat(v_cache[:, :, Sk - W:, :], rep, axis=1)
        scores = jnp.einsum("bhqd,bhkd->bhqk", q, k) * (Dh ** -0.5)
        p = _softmax(scores, axis=-1)
        o = jnp.einsum("bhqk,bhkd->bhqd", p, v)
        return (lambda x, *d: x.transpose(*d))(o, 0, 2, 1, 3).reshape(B, Sq, Hq * Dh) @ wo

    def _B_ref(x, w1, w3, w2):
        gate = jnp.einsum("bsd,df->bsf", x, w1)
        up = jnp.einsum("bsd,df->bsf", x, w3)
        h = _silu(gate) * up
        out = jnp.einsum("bsf,fd->bsd", h, w2)
        return out

    x = A_x
    xn = _layernorm(x, axis=-1)
    s = _A_ref(xn, A_k_cache, A_v_cache, A_wq, A_wo)
    g = _silu(_B_ref(xn, B_w1, B_w3, B_w2))
    return x + s * g
```

```python
import jax
import jax.numpy as jnp
from jax import lax
import jax.experimental.pallas as pl
import jax.experimental.pallas.tpu as pltpu

_HQ = 32
_DH = 192
_EPS = 1e-5
_LANES = 128
_RING = 3
_WROWS = 160
_OROWS = 32


def _silu(z):
    return z * (1.0 / (1.0 + jnp.exp(-z)))


def _kernel(x_hbm, kt_hbm, vt_hbm, wq_hbm, wo_hbm, w1_hbm, w3_hbm, w2_hbm,
            o_ref,
            x_buf, wq_buf, wo_buf, w1_buf, w3_buf, w2_buf, k_buf, v_buf,
            qb_ref, s_ref, p_ref,
            x_sem, wq_sem, wo_sem, w13_sem, w2_sem, k_sem, v_sem,
            *, window, unroll):
    f32, bf16 = jnp.float32, jnp.bfloat16
    d_model = x_buf.shape[1]
    n_heads = kt_hbm.shape[0] // _DH
    col0 = kt_hbm.shape[1] - window
    n_chunks = window // _LANES
    n_qblk = wq_buf.shape[0]
    n_fblk = w1_buf.shape[0]
    w_split = d_model // _WROWS
    n_wo = wo_buf.shape[0] // _OROWS
    n_w2 = w2_buf.shape[0] // _OROWS

    def start_cache(hbm, buf, sem, h, c, queue):
        slot = h % _RING
        src = hbm.at[pl.ds(pl.multiple_of(h * _DH, _DH), _DH),
                     pl.ds(pl.multiple_of(col0 + c * _LANES, _LANES), _LANES)]
        pltpu.make_async_copy(src, buf.at[slot, c], sem.at[slot]).start(priority=queue)

    def wait_cache(buf, sem, h):
        slot = h % _RING
        pltpu.make_async_copy(buf.at[slot], buf.at[slot], sem.at[slot]).wait()

    def start_cols(hbm, buf, sem, j, r, queue):
        rows = pl.ds(r * _WROWS, _WROWS)
        src = hbm.at[rows, pl.ds(pl.multiple_of(j * _LANES, _LANES), _LANES)]
        pltpu.make_async_copy(src, buf.at[j, rows], sem).start(priority=queue)

    def start_rows(hbm, buf, sem, i, queue):
        rows = pl.ds(pl.multiple_of(i * _OROWS, _OROWS), _OROWS)
        pltpu.make_async_copy(hbm.at[rows], buf.at[rows], sem).start(priority=queue)

    def wait_all(buf, sem):
        pltpu.make_async_copy(buf, buf, sem).wait()

    def start_k(h, c, queue):
        start_cache(kt_hbm, k_buf, k_sem, h, c, queue)

    def start_v(h, c, queue):
        start_cache(vt_hbm, v_buf, v_sem, h, c, queue)

    x_copy = pltpu.make_async_copy(x_hbm, x_buf, x_sem)
    x_copy.start(priority=1)

    @pl.loop(0, n_qblk)
    def _(j):
        for r in range(w_split):
            start_cols(wq_hbm, wq_buf, wq_sem, j, r, r % 2)

    @pl.loop(0, n_chunks)
    def _(c):
        start_k(0, c, 0)
        start_v(0, c, 1)

    @pl.loop(0, n_chunks // 2)
    def _(i):
        start_k(1, 2 * i, 0)
        start_k(1, 2 * i + 1, 1)

    x_copy.wait()
    x = x_buf[...].astype(f32)
    xc = x - jnp.mean(x, axis=-1, keepdims=True)
    var = jnp.mean(xc * xc, axis=-1, keepdims=True)
    xn = xc / jnp.sqrt(var + _EPS)
    xn_rows = jnp.broadcast_to(xn, (16, d_model)).astype(bf16)

    wait_all(wq_buf, wq_sem)
    wo_per_blk = n_wo // n_qblk

    @pl.loop(0, n_qblk)
    def _(j):
        for u in range(wo_per_blk):
            start_rows(wo_hbm, wo_buf, wo_sem, j * wo_per_blk + u, u % 2)
        q = jnp.dot(xn_rows, wq_buf[j], preferred_element_type=f32)[0:1]
        q = jnp.broadcast_to(q * (_DH ** -0.5), (_LANES, _LANES))
        qb_ref[pl.ds(pl.multiple_of(j * _LANES, _LANES), _LANES), :] = q.T

    def head_step(h, enqueue, do_k, do_v):
        if do_k:
            wait_cache(k_buf, k_sem, h + 1)
        if do_v:
            wait_cache(v_buf, v_sem, h)
        k_slot, v_slot = (h + 1) % _RING, h % _RING
        q_rows = pl.ds(pl.multiple_of((h + 1) * _DH, _DH), _DH)

        def body(i, acc):
            for u in range(unroll):
                c = i * unroll + u
                enqueue(c)
                if do_k:
                    prod = k_buf[k_slot, c].astype(f32) * qb_ref[q_rows, :]
                    s_ref[pl.ds(c, 1), :] = jnp.sum(prod, axis=0, keepdims=True)
                if do_v:
                    acc = acc + v_buf[v_slot, c].astype(f32) * p_ref[pl.ds(c, 1), :]
            return acc

        init = jnp.zeros((_DH, _LANES), f32) if do_v else None
        return lax.fori_loop(0, n_chunks // unroll, body, init)

    def softmax():
        s = s_ref[...]
        m = jnp.max(jnp.max(s, axis=0, keepdims=True), axis=1, keepdims=True)
        e = jnp.exp(s - m)
        l = jnp.sum(jnp.sum(e, axis=0, keepdims=True), axis=1, keepdims=True)
        p_ref[...] = e / l

    def project(h, acc, out):
        o = jnp.sum(acc, axis=1, keepdims=True)
        w = wo_buf[pl.ds(pl.multiple_of(h * _DH, _DH), _DH), :].astype(f32)
        return out + jnp.sum((w * o).reshape(_DH // 8, 8, d_model), axis=0)

    def enq_kv(h):
        def enqueue(c):
            start_k(h + 3, c, 0)
            start_v(h + 2, c, 1)
        return enqueue

    head_step(-1, enq_kv(-1), True, False)
    softmax()
    wait_all(wo_buf, wo_sem)

    def main(h, out):
        out = project(h, head_step(h, enq_kv(h), True, True), out)
        softmax()
        return out

    out = lax.fori_loop(0, n_heads - 3, main, jnp.zeros((8, d_model), f32))

    n_w13 = n_fblk * w_split

    def start_w13(hbm, buf, i, queue):
        rows = pl.ds(pl.multiple_of((i // n_fblk) * _WROWS, _WROWS), _WROWS)
        j = i % n_fblk
        src = hbm.at[rows, pl.ds(pl.multiple_of(j * _LANES, _LANES), _LANES)]
        pltpu.make_async_copy(src, buf.at[j, rows], w13_sem).start(priority=queue)

    def enq_tail0(c):
        start_w13(w1_hbm, w1_buf, c, 0)
        start_v(n_heads - 1, c, 1)

    def enq_tail1(c):
        rest = n_w13 - n_chunks

        @pl.when(c < rest)
        def _():
            start_w13(w1_hbm, w1_buf, n_chunks + c, 0)

        @pl.when(c >= rest)
        def _():
            start_w13(w3_hbm, w3_buf, n_chunks + c - rest, 0)

        start_w13(w3_hbm, w3_buf, c, 1)

    def enq_tail2(c):
        @pl.when(c < n_w2 // 2)
        def _():
            start_rows(w2_hbm, w2_buf, w2_sem, 2 * c, 0)
            start_rows(w2_hbm, w2_buf, w2_sem, 2 * c + 1, 1)

    h = n_heads - 3
    out = project(h, head_step(h, enq_tail0, True, True), out)
    softmax()
    out = project(h + 1, head_step(h + 1, enq_tail1, True, True), out)
    softmax()
    out = project(h + 2, head_step(h + 2, enq_tail2, False, True), out)
    attn = jnp.sum(out, axis=0, keepdims=True)

    wait_all(w1_buf, w13_sem)
    wait_all(w3_buf, w13_sem)
    hid = []
    for j in range(n_fblk):
        gate = jnp.dot(xn_rows, w1_buf[j], preferred_element_type=f32)
        up = jnp.dot(xn_rows, w3_buf[j], preferred_element_type=f32)
        hid.append((_silu(gate) * up).astype(bf16))
    hid = jnp.concatenate(hid, axis=1)
    wait_all(w2_buf, w2_sem)
    ffn = jnp.dot(hid, w2_buf[...], preferred_element_type=f32)[0:1]
    o_ref[...] = (x + attn * _silu(ffn)).astype(o_ref.dtype)


@jax.jit
def pallas_recurrent_scan__sliding_block_cached__glu_gated_swiglu__decode_kernel(
    A_x: jax.Array,
    A_k_cache: jax.Array,
    A_v_cache: jax.Array,
    A_wq: jax.Array,
    A_wo: jax.Array,
    B_x: jax.Array,
    B_w1: jax.Array,
    B_w3: jax.Array,
    B_w2: jax.Array,
):
    del B_x
    batch, sq, d_model = A_x.shape
    _, n_heads, sk, dh = A_k_cache.shape
    d_ff = B_w1.shape[1]
    window = min(4096, max(256, sk // 4))
    n_chunks = window // _LANES
    assert (batch, sq, n_heads, dh) == (1, 1, _HQ, _DH)
    assert (d_model, d_ff, n_chunks) == (640, 1536, 32) and (sk - window) % _LANES == 0

    kt = jnp.swapaxes(A_k_cache, 2, 3).reshape(n_heads * dh, sk)
    vt = jnp.swapaxes(A_v_cache, 2, 3).reshape(n_heads * dh, sk)

    bf16, f32 = jnp.bfloat16, jnp.float32
    dma = pltpu.SemaphoreType.DMA

    def kernel(*refs):
        _kernel(*refs, window=window, unroll=2)

    out = pl.pallas_call(
        kernel,
        out_shape=jax.ShapeDtypeStruct((1, d_model), A_x.dtype),
        in_specs=[pl.BlockSpec(memory_space=pl.ANY)] * 8,
        out_specs=pl.BlockSpec(memory_space=pltpu.VMEM),
        scratch_shapes=[
            pltpu.VMEM((1, d_model), bf16),
            pltpu.VMEM((n_heads * dh // _LANES, d_model, _LANES), bf16),
            pltpu.VMEM((n_heads * dh, d_model), bf16),
            pltpu.VMEM((d_ff // _LANES, d_model, _LANES), bf16),
            pltpu.VMEM((d_ff // _LANES, d_model, _LANES), bf16),
            pltpu.VMEM((d_ff, d_model), bf16),
            pltpu.VMEM((_RING, n_chunks, dh, _LANES), bf16),
            pltpu.VMEM((_RING, n_chunks, dh, _LANES), bf16),
            pltpu.VMEM((n_heads * dh, _LANES), f32),
            pltpu.VMEM((n_chunks, _LANES), f32),
            pltpu.VMEM((n_chunks, _LANES), f32),
            dma(()), dma(()), dma(()), dma(()), dma(()),
            dma((_RING,)), dma((_RING,)),
        ],
        compiler_params=pltpu.CompilerParams(
            vmem_limit_bytes=64 * 1024 * 1024,
        ),
    )(A_x.reshape(1, d_model), kt, vt, A_wq, A_wo, B_w1, B_w3, B_w2)
    return out.reshape(batch, sq, d_model)
```

```python
import jax
import jax.numpy as jnp
from jax import lax
import jax.experimental.pallas as pl
import jax.experimental.pallas.tpu as pltpu

_HQ = 32
_DH = 192
_EPS = 1e-5
_LANES = 128
_RING = 4
_AHEAD = 2
_WROWS = 160
_OROWS = 32
_W2_PARTS = 6
_QG = 4
_KU = 4
_VU = 4


def _silu(z):
    return z * (1.0 / (1.0 + jnp.exp(-z)))


def _tree_sum(parts):
    while len(parts) > 1:
        parts = [sum(parts[i + 1:i + 2], parts[i]) for i in range(0, len(parts), 2)]
    return parts[0]


def _kernel(x_hbm, kt_hbm, vt_hbm, wq_hbm, wo_hbm, w1_hbm, w3_hbm, w2_hbm,
            o_ref,
            x_buf, wq_buf, wo_buf, w1_buf, w3_buf, w2_buf, k_buf, v_buf,
            qb_ref, s_ref, p_ref,
            x_sem, wq_sem, wo_sem, w1_sem, w3_sem, w2_sem, k_sem, v_sem):
    f32, bf16 = jnp.float32, jnp.bfloat16
    d_model = x_buf.shape[1]
    n_heads = kt_hbm.shape[0] // _DH
    n_chunks = k_buf.shape[1]
    col0 = kt_hbm.shape[1] - n_chunks * _LANES
    n_qblk = wq_buf.shape[0]
    n_fblk = w1_buf.shape[0]
    w_split = d_model // _WROWS
    assert wo_buf.shape[0] == n_qblk * w_split * _OROWS
    w2_rows = w2_buf.shape[0] // _W2_PARTS

    def start_cols(hbm, buf, sem, j, r, queue):
        rows = pl.ds(r * _WROWS, _WROWS)
        src = hbm.at[rows, pl.ds(pl.multiple_of(j * _LANES, _LANES), _LANES)]
        pltpu.make_async_copy(src, buf.at[j, rows], sem).start(priority=queue)

    def start_rows(hbm, buf, sem, i, queue):
        rows = pl.ds(pl.multiple_of(i * _OROWS, _OROWS), _OROWS)
        pltpu.make_async_copy(hbm.at[rows], buf.at[rows], sem).start(priority=queue)

    def start_head(h):
        slot = h % _RING
        rows = pl.ds(pl.multiple_of(h * _DH, _DH), _DH)

        @pl.loop(0, n_chunks)
        def _(c):
            cols = pl.ds(pl.multiple_of(col0 + c * _LANES, _LANES), _LANES)
            pltpu.make_async_copy(kt_hbm.at[rows, cols], k_buf.at[slot, c],
                                  k_sem.at[slot]).start(priority=0)
            pltpu.make_async_copy(vt_hbm.at[rows, cols], v_buf.at[slot, c],
                                  v_sem.at[slot]).start(priority=1)

    def wait_all(buf, sem):
        pltpu.make_async_copy(buf, buf, sem).wait()

    x_copy = pltpu.make_async_copy(x_hbm, x_buf, x_sem)
    x_copy.start(priority=1)

    @pl.loop(0, n_qblk)
    def _(j):
        for r in range(w_split):
            start_cols(wq_hbm, wq_buf, wq_sem, j, r, 0)
            start_rows(wo_hbm, wo_buf, wo_sem, j * w_split + r, 1)

    start_head(0)

    x_copy.wait()
    x = x_buf[...].astype(f32)
    xc = x - jnp.mean(x, axis=-1, keepdims=True)
    var = jnp.mean(xc * xc, axis=-1, keepdims=True)
    xn = xc / jnp.sqrt(var + _EPS)
    xn_rows = jnp.broadcast_to(xn, (16, d_model)).astype(bf16)

    def q_group(g):
        for u in range(_QG):
            j = g * _QG + u
            q = jnp.dot(xn_rows, wq_buf[j], preferred_element_type=f32)[0:1]
            q = jnp.broadcast_to(q * (_DH ** -0.5), (_LANES, _LANES))
            qb_ref[pl.ds(pl.multiple_of(j * _LANES, _LANES), _LANES), :] = q.T

    for h in range(1, _AHEAD):
        start_head(h)
    wait_all(wq_buf, wq_sem)
    q_group(0)
    wait_all(wo_buf, wo_sem)

    def attend(h, out):
        slot = h % _RING
        rows = pl.ds(pl.multiple_of(h * _DH, _DH), _DH)

        wait_all(k_buf.at[slot], k_sem.at[slot])
        q = qb_ref[rows, :]

        @pl.loop(0, n_chunks // _KU)
        def _(i):
            for u in range(_KU):
                c = i * _KU + u
                prod = k_buf[slot, c].astype(f32) * q
                part = _tree_sum([prod[r:r + 8] for r in range(0, _DH, 8)])
                s_ref[pl.ds(c, 1), :] = jnp.sum(part, axis=0, keepdims=True)

        s = s_ref[...]
        m = jnp.max(jnp.max(s, axis=0, keepdims=True), axis=1, keepdims=True)
        e = jnp.exp(s - m)
        p_ref[...] = e
        denom = jnp.sum(jnp.sum(e, axis=0, keepdims=True), axis=1, keepdims=True)

        wait_all(v_buf.at[slot], v_sem.at[slot])

        def values(i, acc):
            for u in range(_VU):
                c = i * _VU + u
                acc = acc + v_buf[slot, c].astype(f32) * p_ref[pl.ds(c, 1), :]
            return acc

        acc = lax.fori_loop(0, n_chunks // _VU, values, jnp.zeros((_DH, _LANES), f32))
        o = jnp.sum(acc, axis=1, keepdims=True) / denom
        prod = wo_buf[rows, :].astype(f32) * o
        return out + _tree_sum([prod[r:r + 8] for r in range(0, _DH, 8)])

    def step(h, out):
        start_head(h + _AHEAD)
        pl.when(h + 1 < n_qblk // _QG)(lambda: q_group(h + 1))
        return attend(h, out)

    out = lax.fori_loop(0, n_heads - _AHEAD, step, jnp.zeros((8, d_model), f32))

    @pl.loop(0, n_fblk)
    def _(j):
        for r in range(w_split):
            start_cols(w1_hbm, w1_buf, w1_sem, j, r, 0)
            start_cols(w3_hbm, w3_buf, w3_sem, j, r, 1)

    for h in range(n_heads - _AHEAD, n_heads - 1):
        out = attend(h, out)

    @pl.loop(0, _W2_PARTS)
    def _(part):
        for u in range(w2_rows // _OROWS):
            start_rows(w2_hbm, w2_buf, w2_sem.at[part],
                       part * (w2_rows // _OROWS) + u, u % 2)

    out = attend(n_heads - 1, out)
    attn = jnp.sum(out, axis=0, keepdims=True)

    wait_all(w1_buf, w1_sem)
    wait_all(w3_buf, w3_sem)
    hid = []
    for j in range(n_fblk):
        gate = jnp.dot(xn_rows, w1_buf[j], preferred_element_type=f32)
        up = jnp.dot(xn_rows, w3_buf[j], preferred_element_type=f32)
        hid.append((_silu(gate) * up).astype(bf16))
    hid = jnp.concatenate(hid, axis=1)

    ffn = jnp.zeros((16, d_model), f32)
    for part in range(_W2_PARTS):
        rows = pl.ds(part * w2_rows, w2_rows)
        wait_all(w2_buf.at[rows], w2_sem.at[part])
        ffn = ffn + jnp.dot(hid[:, part * w2_rows:(part + 1) * w2_rows],
                            w2_buf[rows, :], preferred_element_type=f32)
    o_ref[...] = (x + attn * _silu(ffn[0:1])).astype(o_ref.dtype)


@jax.jit
def pallas_recurrent_scan__sliding_block_cached__glu_gated_swiglu__decode_kernel(
    A_x: jax.Array,
    A_k_cache: jax.Array,
    A_v_cache: jax.Array,
    A_wq: jax.Array,
    A_wo: jax.Array,
    B_x: jax.Array,
    B_w1: jax.Array,
    B_w3: jax.Array,
    B_w2: jax.Array,
):
    del B_x
    batch, sq, d_model = A_x.shape
    _, n_heads, sk, dh = A_k_cache.shape
    d_ff = B_w1.shape[1]
    window = min(4096, max(256, sk // 4))
    n_chunks = window // _LANES
    assert (batch, sq, n_heads, dh) == (1, 1, _HQ, _DH)
    assert (d_model, d_ff) == (640, 1536)
    assert window % (_LANES * 8) == 0 and sk % _LANES == 0

    kt = jnp.swapaxes(A_k_cache, 2, 3).reshape(n_heads * dh, sk)
    vt = jnp.swapaxes(A_v_cache, 2, 3).reshape(n_heads * dh, sk)

    bf16, f32 = jnp.bfloat16, jnp.float32
    dma = pltpu.SemaphoreType.DMA
    out = pl.pallas_call(
        _kernel,
        out_shape=jax.ShapeDtypeStruct((1, d_model), A_x.dtype),
        in_specs=[pl.BlockSpec(memory_space=pl.ANY)] * 8,
        out_specs=pl.BlockSpec(memory_space=pltpu.VMEM),
        scratch_shapes=[
            pltpu.VMEM((1, d_model), bf16),
            pltpu.VMEM((n_heads * dh // _LANES, d_model, _LANES), bf16),
            pltpu.VMEM((n_heads * dh, d_model), bf16),
            pltpu.VMEM((d_ff // _LANES, d_model, _LANES), bf16),
            pltpu.VMEM((d_ff // _LANES, d_model, _LANES), bf16),
            pltpu.VMEM((d_ff, d_model), bf16),
            pltpu.VMEM((_RING, n_chunks, dh, _LANES), bf16),
            pltpu.VMEM((_RING, n_chunks, dh, _LANES), bf16),
            pltpu.VMEM((n_heads * dh, _LANES), f32),
            pltpu.VMEM((n_chunks, _LANES), f32),
            pltpu.VMEM((n_chunks, _LANES), f32),
            dma(()), dma(()), dma(()), dma(()), dma(()),
            dma((_W2_PARTS,)), dma((_RING,)), dma((_RING,)),
        ],
        compiler_params=pltpu.CompilerParams(
            vmem_limit_bytes=64 * 1024 * 1024,
        ),
    )(A_x.reshape(1, d_model), kt, vt, A_wq, A_wo, B_w1, B_w3, B_w2)
    return out.reshape(batch, sq, d_model)
```

```python
import jax
import jax.numpy as jnp
from jax import lax
import jax.experimental.pallas as pl
import jax.experimental.pallas.tpu as pltpu

_HQ = 32
_DH = 192
_EPS = 1e-5
_LANES = 128
_AHEAD = 2
_RING = 3
_CROWS = 160
_RROWS = 32
_W2_PARTS = 3
_QG = 4
_FG = 2
_UNROLL = 4


def _fold_rows(a):
    parts = [a[r:r + 8] for r in range(0, a.shape[0], 8)]
    while len(parts) > 1:
        parts = [sum(parts[i + 1:i + 2], parts[i]) for i in range(0, len(parts), 2)]
    return parts[0]


def _kernel(x_hbm, kt_hbm, vt_hbm, wq_hbm, wo_hbm, w1_hbm, w3_hbm, w2_hbm,
            o_ref,
            x_buf, wc_buf, wo_buf, w2_buf, k_buf, v_buf, qb_ref, hid_ref, s_ref, p_ref,
            w_sem, k_sem, v_sem):
    f32, bf16 = jnp.float32, jnp.bfloat16
    d_model = x_buf.shape[1]
    n_heads = kt_hbm.shape[0] // _DH
    n_chunks = k_buf.shape[1]
    col0 = kt_hbm.shape[1] - n_chunks * _LANES
    n_qblk = wq_hbm.shape[1] // _LANES
    n_fblk = w1_hbm.shape[1] // _LANES
    c_split = d_model // _CROWS
    w2_rows = w2_buf.shape[0] // _W2_PARTS
    n_qgrp, n_fgrp = n_qblk // _QG, n_fblk // _FG
    assert wo_buf.shape[0] == n_qblk * c_split * _RROWS
    assert _QG * _LANES >= _DH and n_qgrp + n_fgrp <= n_heads - _AHEAD

    def start_cols(hbm, base, j, r, queue):
        rows = pl.ds(r * _CROWS, _CROWS)
        src = hbm.at[rows, pl.ds(pl.multiple_of(j * _LANES, _LANES), _LANES)]
        pltpu.make_async_copy(src, wc_buf.at[base + j, rows],
                              w_sem.at[0]).start(priority=queue)

    def start_rows(hbm, buf, sem, i, queue):
        rows = pl.ds(pl.multiple_of(i * _RROWS, _RROWS), _RROWS)
        pltpu.make_async_copy(hbm.at[rows], buf.at[rows], sem).start(priority=queue)

    def start_head(h):
        slot = h % _RING
        rows = pl.ds(pl.multiple_of(h * _DH, _DH), _DH)

        @pl.loop(0, n_chunks)
        def _(c):
            cols = pl.ds(pl.multiple_of(col0 + c * _LANES, _LANES), _LANES)
            pltpu.make_async_copy(kt_hbm.at[rows, cols], k_buf.at[slot, c],
                                  k_sem.at[slot]).start(priority=0)
            pltpu.make_async_copy(vt_hbm.at[rows, cols], v_buf.at[slot, c],
                                  v_sem.at[slot]).start(priority=1)

    def wait_all(buf, sem):
        pltpu.make_async_copy(buf, buf, sem).wait()

    x_copy = pltpu.make_async_copy(x_hbm, x_buf, w_sem.at[2])
    x_copy.start()

    @pl.loop(0, n_qblk)
    def _(j):
        for r in range(c_split):
            start_cols(wq_hbm, 0, j, r, 0)
            start_rows(wo_hbm, wo_buf, w_sem.at[1], j * c_split + r, 1)

    @pl.loop(0, n_fblk)
    def _(j):
        for r in range(c_split):
            start_cols(w1_hbm, n_qblk, j, r, 0)
            start_cols(w3_hbm, n_qblk + n_fblk, j, r, 1)

    x_copy.wait()
    x = x_buf[...].astype(f32)
    xc = x - jnp.mean(x, axis=-1, keepdims=True)
    var = jnp.mean(xc * xc, axis=-1, keepdims=True)
    xn = xc / jnp.sqrt(var + _EPS)
    xn_rows = jnp.broadcast_to(xn, (16, d_model)).astype(bf16)

    def project_xn(block):
        return jnp.dot(xn_rows, wc_buf[block], preferred_element_type=f32)

    def q_group(g):
        for u in range(_QG):
            j = g * _QG + u
            q = jnp.broadcast_to(project_xn(j)[0:1] * (_DH ** -0.5), (_LANES, _LANES))
            qb_ref[pl.ds(pl.multiple_of(j * _LANES, _LANES), _LANES), :] = q.T

    def ffn_group(g):
        for u in range(_FG):
            j = g * _FG + u
            gate, up = project_xn(n_qblk + j), project_xn(n_qblk + n_fblk + j)
            hid_ref[j] = (jax.nn.silu(gate) * up).astype(bf16)

    pl.loop(0, _AHEAD)(start_head)
    wait_all(wc_buf, w_sem.at[0])
    wait_all(wo_buf, w_sem.at[1])

    def attend(h, out):
        slot = h % _RING
        rows = pl.ds(pl.multiple_of(h * _DH, _DH), _DH)
        wait_all(k_buf.at[slot], k_sem.at[slot])
        q = qb_ref[rows, :]

        @pl.loop(0, n_chunks // _UNROLL)
        def _(i):
            for u in range(_UNROLL):
                c = i * _UNROLL + u
                part = _fold_rows(k_buf[slot, c].astype(f32) * q)
                s_ref[pl.ds(c, 1), :] = jnp.sum(part, axis=0, keepdims=True)

        s = s_ref[...]
        m = jnp.max(jnp.max(s, axis=0, keepdims=True), axis=1, keepdims=True)
        e = jnp.exp(s - m)
        p_ref[...] = e
        denom = jnp.sum(jnp.sum(e, axis=0, keepdims=True), axis=1, keepdims=True)

        wait_all(v_buf.at[slot], v_sem.at[slot])

        def values(i, acc):
            for u in range(_UNROLL):
                c = i * _UNROLL + u
                acc = acc + v_buf[slot, c].astype(f32) * p_ref[pl.ds(c, 1), :]
            return acc

        acc = lax.fori_loop(0, n_chunks // _UNROLL, values,
                            jnp.zeros((_DH, _LANES), f32))
        o = jnp.sum(acc, axis=1, keepdims=True) / denom
        return out + _fold_rows(wo_buf[rows, :].astype(f32) * o)

    def step(h, out):
        start_head(h + _AHEAD)
        pl.when(h < n_qgrp)(lambda: q_group(h))
        pl.when((h >= n_qgrp) & (h < n_qgrp + n_fgrp))(lambda: ffn_group(h - n_qgrp))
        return attend(h, out)

    out = lax.fori_loop(0, n_heads - _AHEAD, step, jnp.zeros((8, d_model), f32))

    @pl.loop(0, _W2_PARTS)
    def _(part):
        for u in range(w2_rows // _RROWS):
            start_rows(w2_hbm, w2_buf, w_sem.at[part],
                       part * (w2_rows // _RROWS) + u, u % 2)

    out = lax.fori_loop(n_heads - _AHEAD, n_heads, attend, out)
    attn = jnp.sum(out, axis=0, keepdims=True)

    ffn = jnp.zeros((16, d_model), f32)
    for part in range(_W2_PARTS):
        lo, hi = part * w2_rows, (part + 1) * w2_rows
        hid = jnp.concatenate(
            [hid_ref[j] for j in range(lo // _LANES, hi // _LANES)], axis=1)
        wait_all(w2_buf.at[pl.ds(lo, w2_rows)], w_sem.at[part])
        ffn = ffn + jnp.dot(hid, w2_buf[lo:hi, :], preferred_element_type=f32)
    o_ref[...] = (x + attn * jax.nn.silu(ffn[0:1])).astype(o_ref.dtype)


@jax.jit
def pallas_recurrent_scan__sliding_block_cached__glu_gated_swiglu__decode_kernel(
    A_x: jax.Array,
    A_k_cache: jax.Array,
    A_v_cache: jax.Array,
    A_wq: jax.Array,
    A_wo: jax.Array,
    B_x: jax.Array,
    B_w1: jax.Array,
    B_w3: jax.Array,
    B_w2: jax.Array,
):
    del B_x
    batch, sq, d_model = A_x.shape
    _, n_heads, sk, dh = A_k_cache.shape
    d_ff = B_w1.shape[1]
    window = min(4096, max(256, sk // 4))
    n_chunks = window // _LANES
    assert (batch, sq, n_heads, dh, d_model, d_ff) == (1, 1, _HQ, _DH, 640, 1536)
    assert window % (8 * _LANES) == 0 and sk % _LANES == 0

    kt = jnp.swapaxes(A_k_cache, 2, 3).reshape(n_heads * dh, sk)
    vt = jnp.swapaxes(A_v_cache, 2, 3).reshape(n_heads * dh, sk)

    bf16, f32 = jnp.bfloat16, jnp.float32
    n_cblk = (n_heads * dh + 2 * d_ff) // _LANES
    out = pl.pallas_call(
        _kernel,
        out_shape=jax.ShapeDtypeStruct((1, d_model), A_x.dtype),
        in_specs=[pl.BlockSpec(memory_space=pl.ANY)] * 8,
        out_specs=pl.BlockSpec(memory_space=pltpu.VMEM),
        scratch_shapes=[
            pltpu.VMEM((1, d_model), bf16),
            pltpu.VMEM((n_cblk, d_model, _LANES), bf16),
            pltpu.VMEM((n_heads * dh, d_model), bf16),
            pltpu.VMEM((d_ff, d_model), bf16),
            pltpu.VMEM((_RING, n_chunks, dh, _LANES), bf16),
            pltpu.VMEM((_RING, n_chunks, dh, _LANES), bf16),
            pltpu.VMEM((n_heads * dh, _LANES), f32),
            pltpu.VMEM((d_ff // _LANES, 16, _LANES), bf16),
            pltpu.VMEM((n_chunks, _LANES), f32),
            pltpu.VMEM((n_chunks, _LANES), f32),
            pltpu.SemaphoreType.DMA((_W2_PARTS,)),
            pltpu.SemaphoreType.DMA((_RING,)),
            pltpu.SemaphoreType.DMA((_RING,)),
        ],
        compiler_params=pltpu.CompilerParams(vmem_limit_bytes=64 * 1024 * 1024),
    )(A_x.reshape(1, d_model), kt, vt, A_wq, A_wo, B_w1, B_w3, B_w2)
    return out.reshape(batch, sq, d_model)
```
